```python
import jax
import jax.numpy as jnp

def _softmax(x, axis=-1):
    return jax.nn.softmax(x, axis=axis)
def _gelu(x):
    return jax.nn.gelu(x, approximate=True)
def _silu(x):
    return jax.nn.silu(x)
def _sigmoid(x):
    return jax.nn.sigmoid(x)
def _layernorm(x, axis=-1, eps=1e-5):
    m = jnp.mean(x, axis=axis, keepdims=True)
    v = jnp.var(x, axis=axis, keepdims=True)
    return (x - m) / jnp.sqrt(v + eps)
def _scatter_add(tgt, idx, src, axis=0):
    return tgt.at[idx].add(src)
def _segment_sum(src, seg, n):
    return jax.ops.segment_sum(src, seg, n)
class _Rng:
    def __init__(self, key):
        self._k = key
    def _next(self):
        self._k, sub = jax.random.split(self._k)
        return sub
    def normal(self, shape):
        return jax.random.normal(self._next(), shape, dtype=jnp.bfloat16)
    def randint(self, lo, hi, shape):
        return jax.random.randint(self._next(), shape, lo, hi, dtype=jnp.int32)
    def uniform(self, shape, lo=0.0, hi=1.0):
        return jax.random.uniform(self._next(), shape, jnp.bfloat16, lo, hi)
    def permutation(self, n):
        return jax.random.permutation(self._next(), n)


kernel_name = 'parallel_sum__ssm_conv_s5__moe_arch_mod__prompt'

def setup_inputs():
    _rng = _Rng(jax.random.key(int.from_bytes(__import__("os").urandom(4), "little")))
    _w = (lambda a: (lambda t: t.astype(jnp.bfloat16) if jnp.issubdtype(t.dtype, jnp.floating) else t)(jnp.asarray(a)))
    def _A_setup():
        B, S, D = 1, 2048, 1024
        P = D
        Lambda_re = -0.5 * jnp.exp((lambda *s: _rng.normal(s) * 0.05)(P))
        Lambda_im = (lambda *s: _rng.normal(s) * 0.05)(P) * 1.0
        B_re = (lambda *s: _rng.normal(s) * 0.05)(P, D) * (D ** -0.5)
        B_im = (lambda *s: _rng.normal(s) * 0.05)(P, D) * (D ** -0.5)
        C_re = (lambda *s: _rng.normal(s) * 0.05)(D, P) * (P ** -0.5)
        C_im = (lambda *s: _rng.normal(s) * 0.05)(D, P) * (P ** -0.5)
        log_dt = (lambda *s: _rng.normal(s) * 0.05)(P) * 0.3 - 2.0
        Dskip = (lambda *s: _rng.normal(s) * 0.05)(D)
        return {
            "x": _w((lambda *s: _rng.normal(s) * 0.05)(B, S, D)),
            "Lambda_re": _w(Lambda_re),
            "Lambda_im": _w(Lambda_im),
            "B_re": _w(B_re),
            "B_im": _w(B_im),
            "C_re": _w(C_re),
            "C_im": _w(C_im),
            "log_dt": _w(log_dt),
            "Dskip": _w(Dskip),
        }
    _A_in = _A_setup()

    def _B_setup():
        B, S, D, F, C = 1, 2048, 1024, 3584, 2
        return {
            "x": _w((lambda *s: _rng.normal(s) * 0.05)(B, S, D)),
            "w_r": _w((lambda *s: _rng.normal(s) * 0.05)(D)),
            "w_gate": _w((lambda *s: _rng.normal(s) * 0.05)(D, F)),
            "w_up": _w((lambda *s: _rng.normal(s) * 0.05)(D, F)),
            "w_down": _w((lambda *s: _rng.normal(s) * 0.05)(F, D)),
        }
    _B_in = _B_setup()

    return {
        "A_x": _A_in["x"],
        "A_Lambda_re": _A_in["Lambda_re"],
        "A_Lambda_im": _A_in["Lambda_im"],
        "A_B_re": _A_in["B_re"],
        "A_B_im": _A_in["B_im"],
        "A_C_re": _A_in["C_re"],
        "A_C_im": _A_in["C_im"],
        "A_log_dt": _A_in["log_dt"],
        "A_Dskip": _A_in["Dskip"],
        "B_x": _B_in["x"],
        "B_w_r": _B_in["w_r"],
        "B_w_gate": _B_in["w_gate"],
        "B_w_up": _B_in["w_up"],
        "B_w_down": _B_in["w_down"],
    }

def reference(A_x, A_Lambda_re, A_Lambda_im, A_B_re, A_B_im, A_C_re, A_C_im, A_log_dt, A_Dskip, B_x, B_w_r, B_w_gate, B_w_up, B_w_down):
    def _A_ref(x, Lambda_re, Lambda_im, B_re, B_im, C_re, C_im, log_dt, Dskip):
        Bsz, L, H = x.shape
        Lam = Lambda_re + 1j * Lambda_im
        Bmat = B_re + 1j * B_im
        Cmat = C_re + 1j * C_im
        dt = jnp.exp(log_dt)
        Lam_bar = jnp.exp(dt * Lam)
        B_bar = ((Lam_bar - 1.0) / Lam)[:, None] * Bmat
        Bu = jnp.einsum("bld,pd->blp", x + 0j, B_bar)
        h = jnp.zeros_like(Bu[:, 0, :])
        hs = []
        for t in range(L):
            h = Lam_bar[None, :] * h + Bu[:, t, :]
            hs.append(h)
        hseq = jnp.stack(hs, 1)
        y = 2.0 * jnp.einsum("blp,dp->bld", hseq, Cmat).real + x * Dskip[None, None, :]
        return y

    def _B_ref(x, w_r, w_gate, w_up, w_down):
        B, S, D = x.shape
        C = 2
        r = x @ w_r
        idx = jnp.argsort(-r, axis=-1)[:, :C]
        idx_e = jnp.repeat(idx.reshape(B, C, 1), D, axis=2)
        x_sel = jnp.take_along_axis(x, idx_e, axis=1)
        g = _silu(x_sel @ w_gate)
        u = x_sel @ w_up
        y = (g * u) @ w_down
        r_sel = _sigmoid(jnp.take_along_axis(r, idx, axis=1))
        y = y * r_sel.reshape(B, C, 1)
        b_off = (jnp.arange(B) * S).reshape(B, 1)
        flat_idx = (idx + b_off).reshape(B * C)
        zero = (x * 0.0).reshape(B * S, D)
        upd = _scatter_add(zero, flat_idx, y.reshape(B * C, D), axis=0)
        return x + upd.reshape(B, S, D)

    x = A_x
    xn = _layernorm(x, axis=-1)
    return x + _A_ref(xn, A_Lambda_re, A_Lambda_im, A_B_re, A_B_im, A_C_re, A_C_im, A_log_dt, A_Dskip) + _B_ref(xn, B_w_r, B_w_gate, B_w_up, B_w_down)
```

```python
import jax
import jax.numpy as jnp
from jax import lax
import jax.experimental.pallas as pl
import jax.experimental.pallas.tpu as pltpu

S, D, P, F = 2048, 1024, 1024, 3584
NC = 8
LC = S // NC
NB = 8
TI = LC // NB
MB = TI * NC
NL = D // 128
NF = 4
FP = F // NF
FT = FP // 128
f32, bf16, u32 = jnp.float32, jnp.bfloat16, jnp.uint32
NT_DIMS = (((1,), (1,)), ((), ()))


def _rb(v):
    return v.astype(bf16).astype(f32)


def _unpack(w):
    u = pltpu.bitcast(w, u32)
    return pltpu.bitcast(u << 16, f32), pltpu.bitcast(u & jnp.uint32(0xFFFF0000), f32)


def _kernel(lre_ref, lim_ref, ldt_ref, dsk_ref, wr_ref,
            x_hbm, bre_hbm, bim_hbm, cre_hbm, cim_hbm, wg_hbm, wu_hbm, wd_hbm,
            o_hbm,
            x_v, b_v, c_v, wg_v, wu_v, wd_v, xp_v, t_v, bu_v, h_v, o_v, r_v, st_v, lam_v,
            xb_v, ab_v, acc_v, sem_x, sem_w, sem_o):
    def x_cp(k):
        return pltpu.make_async_copy(x_hbm.at[:, pl.ds(k * TI, TI), :], x_v.at[k], sem_x.at[k])

    def o_cp(k):
        return pltpu.make_async_copy(o_v.at[k], o_hbm.at[:, pl.ds(k * TI, TI), :], sem_o.at[k])

    w_cps = [
        pltpu.make_async_copy(bre_hbm, b_v.at[pl.ds(0, P)], sem_w.at[0]),
        pltpu.make_async_copy(bim_hbm, b_v.at[pl.ds(P, P)], sem_w.at[1]),
        pltpu.make_async_copy(cre_hbm, c_v.at[:, pl.ds(0, P)], sem_w.at[2]),
        pltpu.make_async_copy(cim_hbm, c_v.at[:, pl.ds(P, P)], sem_w.at[3]),
    ]

    def wg_cp(i):
        return pltpu.make_async_copy(wg_hbm.at[:, pl.ds(i * FP, FP)], wg_v.at[i], sem_w.at[4 + i])

    def wu_cp(i):
        return pltpu.make_async_copy(wu_hbm.at[:, pl.ds(i * FP, FP)], wu_v.at[i], sem_w.at[4 + NF + i])

    def wd_cp(i):
        return pltpu.make_async_copy(wd_hbm.at[pl.ds(i * FP, FP)], wd_v.at[i], sem_w.at[4 + 2 * NF + i])

    x_cp(0).start()
    w_cps[0].start()
    w_cps[1].start()
    for k in range(1, NB):
        x_cp(k).start()
    w_cps[2].start()
    w_cps[3].start()
    for i in range(NF):
        wg_cp(i).start()
        wu_cp(i).start()
    for i in range(NF):
        wd_cp(i).start()

    row = lambda ref: ref[...].astype(f32).reshape(1, D)
    lre, lim = row(lre_ref), row(lim_ref)
    dt = _rb(jnp.exp(row(ldt_ref)))
    dsk, wr = row(dsk_ref), row(wr_ref)
    mag = jnp.exp(dt * lre)
    ar, ai = mag * jnp.cos(dt * lim), mag * jnp.sin(dt * lim)
    den = lre * lre + lim * lim
    cr = 2.0 * ((ar - 1.0) * lre + ai * lim) / den
    ci = 2.0 * (ai * lre - (ar - 1.0) * lim) / den
    lam_v[0] = jnp.broadcast_to(ar, (8, P))
    lam_v[1] = jnp.broadcast_to(ai, (8, P))
    st_v[...] = jnp.zeros(st_v.shape, f32)

    def ln(k):
        for c in range(NC):
            x = x_v[k, c].astype(f32)
            m = jnp.mean(x, axis=-1, keepdims=True)
            xc = x - m
            v = _rb(jnp.mean(xc * xc, axis=-1, keepdims=True))
            sd = _rb(jnp.sqrt(_rb(v + 1e-5)))
            xn = _rb(_rb(x - _rb(m)) / sd)
            o_v[k, c] = x + xn + xn * dsk
            r = _rb(jnp.sum(xn * wr, axis=-1, keepdims=True))
            r_v[k, c] = jnp.broadcast_to(r, (TI, 128))
            for g in range(TI // 8):
                for j in range(NL):
                    t_v[j, pl.ds(g * 64 + c * 8, 8), :] = xn[g * 8:(g + 1) * 8, j * 128:(j + 1) * 128]
        for g in range(TI // 8):
            for s in range(0, 8, 2):
                for j in range(NL):
                    a = t_v[j, pl.ds(g * 64 + s, 8, stride=8), :]
                    b = t_v[j, pl.ds(g * 64 + s + 1, 8, stride=8), :]
                    xp_v[k, pl.ds(g * 64 + s * 8, 16), pl.ds(j * 128, 128)] = (
                        jnp.concatenate([a, b], axis=0).astype(bf16))

    def mm1(k):
        bu_v[k] = lax.dot_general(xp_v[k], b_v[...], NT_DIMS, preferred_element_type=f32)

    def scan(k, slot=None):
        G = 4
        for j0 in range(0, NL, G):
            js = range(j0, j0 + G)
            lr = [lam_v[0, :, pl.ds(j * 128, 128)] for j in js]
            li = [lam_v[1, :, pl.ds(j * 128, 128)] for j in js]
            hr = [st_v[0, :, pl.ds(j * 128, 128)] for j in js]
            hi = [st_v[1, :, pl.ds(j * 128, 128)] for j in js]
            for i in range(0, TI, 2):
                for n, j in enumerate(js):
                    outr, outi = [], []
                    for ii in (i, i + 1):
                        br = bu_v[k, pl.ds(ii * 8, 8), pl.ds(j * 128, 128)]
                        bi = bu_v[k, pl.ds(ii * 8, 8), pl.ds(P + j * 128, 128)]
                        nr = (lr[n] * hr[n] - li[n] * hi[n]) + br
                        ni = (lr[n] * hi[n] + li[n] * hr[n]) + bi
                        hr[n], hi[n] = nr, ni
                        outr.append(nr)
                        outi.append(ni)
                    if slot is not None:
                        h_v[slot, pl.ds(i * 8, 16), pl.ds(j * 128, 128)] = jnp.concatenate(outr, 0).astype(bf16)
                        h_v[slot, pl.ds(i * 8, 16), pl.ds(P + j * 128, 128)] = jnp.concatenate(outi, 0).astype(bf16)
            for n, j in enumerate(js):
                st_v[0, :, pl.ds(j * 128, 128)] = hr[n]
                st_v[1, :, pl.ds(j * 128, 128)] = hi[n]

    def scale_c(k):
        rows = pl.ds(pl.multiple_of(k * (D // NB), D // NB), D // NB)
        a = c_v[rows, pl.ds(0, P)].astype(f32)
        b = c_v[rows, pl.ds(P, P)].astype(f32)
        c_v[rows, pl.ds(0, P)] = (a * cr - b * ci).astype(bf16)
        c_v[rows, pl.ds(P, P)] = (-(a * ci + b * cr)).astype(bf16)

    def carries():
        pr, pi_ = lam_v[0], lam_v[1]
        n = LC
        while n > 1:
            pr, pi_ = pr * pr - pi_ * pi_, 2.0 * pr * pi_
            n //= 2
        er, ei = st_v[0], st_v[1]
        first = lax.broadcasted_iota(jnp.int32, (8, P), 0) == 0
        sr, si = jnp.zeros_like(er), jnp.zeros_like(ei)
        for _ in range(NC - 1):
            tr = er + (pr * sr - pi_ * si)
            ti = ei + (pr * si + pi_ * sr)
            sr = jnp.where(first, 0.0, pltpu.roll(tr, 1, 0))
            si = jnp.where(first, 0.0, pltpu.roll(ti, 1, 0))
        st_v[0] = sr
        st_v[1] = si

    def mm2(k, slot):
        y = lax.dot_general(h_v[slot], c_v[...], NT_DIMS, preferred_element_type=f32)
        for j in range(NL):
            t_v[j] = y[:, j * 128:(j + 1) * 128]
        for c in range(NC):
            for g in range(TI // 8):
                for j in range(NL):
                    idx = (k, c, pl.ds(g * 8, 8), pl.ds(j * 128, 128))
                    o_v[idx] = o_v[idx] + t_v[j, pl.ds(g * 64 + c, 8, stride=8), :]

    def route():
        r = r_v[...].reshape(S, 128)
        q = lax.broadcasted_iota(jnp.int32, (S, 128), 0)
        tok = ((q // TI) % NC) * LC + (q // MB) * TI + q % TI
        m0 = jnp.max(r, axis=0, keepdims=True)
        i0 = jnp.min(jnp.where(r == m0, tok, S), axis=0, keepdims=True)
        r1 = jnp.where(tok == i0, -jnp.inf, r)
        m1 = jnp.max(r1, axis=0, keepdims=True)
        i1 = jnp.min(jnp.where((r1 == m1) & (tok != i0), tok, S), axis=0, keepdims=True)
        toks = [jnp.clip(jnp.max(i), 0, S - 1) for i in (i0, i1)]
        for n, t in enumerate(toks):
            c, s = t // LC, t % LC
            pr = (s % TI) * 8 + c
            base = pl.multiple_of((pr // 16) * 16, 16)
            tile = xp_v[s // TI, pl.ds(base, 16), :].astype(f32)
            sel = lax.broadcasted_iota(jnp.int32, (16, D), 0) == pr % 16
            xs = jnp.sum(jnp.where(sel, tile, 0.0), axis=0, keepdims=True)
            for j in range(NL):
                xb_v[n, pl.ds(j * 128, 128), :] = jnp.broadcast_to(xs[:, j * 128:(j + 1) * 128], (128, 128)).T
        gates = [_rb(jax.nn.sigmoid(m)) for m in (m0, m1)]
        return toks, gates

    def vecmat(w_ref, i, nk, nt, src, off):
        acc = [[None] * nt for _ in range(2)]
        for kt in range(nk):
            xe = [src[n, pl.ds(off + kt * 16, 8, stride=2), :] for n in range(2)]
            xo = [src[n, pl.ds(off + kt * 16 + 1, 8, stride=2), :] for n in range(2)]
            for j in range(nt):
                we, wo = _unpack(w_ref[i, pl.ds(kt * 16, 16), pl.ds(j * 128, 128)])
                for n in range(2):
                    t = we * xe[n] + wo * xo[n]
                    acc[n][j] = t if acc[n][j] is None else acc[n][j] + t
        return acc

    def ffn_up(i):
        g = vecmat(wg_v, i, D // 16, FT, xb_v, 0)
        u = vecmat(wu_v, i, D // 16, FT, xb_v, 0)
        for n in range(2):
            for j in range(FT):
                gj = _rb(jnp.sum(g[n][j], axis=0, keepdims=True))
                uj = _rb(jnp.sum(u[n][j], axis=0, keepdims=True))
                a = _rb(_rb(gj * jax.nn.sigmoid(gj)) * uj)
                ab_v[n, i, pl.ds(j * 128, 128), :] = jnp.broadcast_to(a, (128, 128)).T

    def ffn_down(i):
        acc = [[None] * NL for _ in range(2)]
        for kt in range(FP // 16):
            xe = [ab_v[n, i, pl.ds(kt * 16, 8, stride=2), :] for n in range(2)]
            xo = [ab_v[n, i, pl.ds(kt * 16 + 1, 8, stride=2), :] for n in range(2)]
            for j in range(NL):
                we, wo = _unpack(wd_v[i, pl.ds(kt * 16, 16), pl.ds(j * 128, 128)])
                for n in range(2):
                    t = we * xe[n] + wo * xo[n]
                    acc[n][j] = t if acc[n][j] is None else acc[n][j] + t
        for n in range(2):
            for j in range(NL):
                idx = (n, slice(None), pl.ds(j * 128, 128))
                acc_v[idx] = acc_v[idx] + acc[n][j]

    x_cp(0).wait()
    ln(0)
    x_cp(1).wait()
    w_cps[0].wait()
    w_cps[1].wait()
    ln(1)
    mm1(0)
    w_cps[2].wait()
    w_cps[3].wait()

    def p1(k, carry):
        x_cp(k + 1).wait()
        ln(k + 1)
        mm1(k)
        scan(k - 1)
        scale_c(k)
        return carry
    lax.fori_loop(1, NB - 1, p1, 0)
    mm1(NB - 1)
    scan(NB - 2)
    scale_c(0)
    scale_c(NB - 1)
    toks, gates = route()
    acc_v[...] = jnp.zeros(acc_v.shape, f32)
    scan(NB - 1)
    carries()
    scan(0, 0)

    def p2a(k, carry):
        wg_cp(k).wait()
        wu_cp(k).wait()
        scan(k + 1, (k + 1) % 2)
        mm2(k, k % 2)
        ffn_up(k)
        o_cp(k).start()
        return carry
    lax.fori_loop(0, NF, p2a, 0)

    def p2b(k, carry):
        wd_cp(k - NF).wait()
        scan(k + 1, (k + 1) % 2)
        mm2(k, k % 2)
        ffn_down(k - NF)
        o_cp(k).start()
        return carry
    lax.fori_loop(NF, NB - 1, p2b, 0)
    wd_cp(NF - 1).wait()
    mm2(NB - 1, (NB - 1) % 2)
    ffn_down(NF - 1)
    for k in range(NB - 1):
        o_cp(k).wait()
    sub = lax.broadcasted_iota(jnp.int32, (8, D), 0)
    fix = []
    for n, t in enumerate(toks):
        c, s = t // LC, t % LC
        y = _rb(_rb(jnp.sum(acc_v[n], axis=0, keepdims=True)) * gates[n][:, :1])
        r0 = pl.multiple_of(((s % TI) // 8) * 8, 8)
        idx = (s // TI, c, pl.ds(r0, 8), slice(None))
        o_v[idx] = o_v[idx] + jnp.where(sub == s % 8, y, 0.0)
        fix.append((s // TI, pltpu.make_async_copy(
            o_v.at[idx], o_hbm.at[c, pl.ds(pl.multiple_of((s // 8) * 8, 8), 8), :], sem_o.at[NB + n]), t // 8))
    o_cp(NB - 1).start()
    do0 = fix[0][0] != NB - 1
    do1 = (fix[1][0] != NB - 1) & (fix[1][2] != fix[0][2])
    pl.when(do0)(lambda: fix[0][1].start())
    pl.when(do1)(lambda: fix[1][1].start())
    pl.when(do0)(lambda: fix[0][1].wait())
    pl.when(do1)(lambda: fix[1][1].wait())
    o_cp(NB - 1).wait()


@jax.jit
def pallas_parallel_sum__ssm_conv_s5__moe_arch_mod__prompt_kernel(
    A_x, A_Lambda_re, A_Lambda_im, A_B_re, A_B_im, A_C_re, A_C_im, A_log_dt, A_Dskip,
    B_x, B_w_r, B_w_gate, B_w_up, B_w_down,
):
    del B_x
    vm = pl.BlockSpec(memory_space=pltpu.VMEM)
    hb = pl.BlockSpec(memory_space=pl.ANY)
    out = pl.pallas_call(
        _kernel,
        out_shape=jax.ShapeDtypeStruct((NC, LC, D), f32),
        in_specs=[vm] * 5 + [hb] * 8,
        out_specs=hb,
        scratch_shapes=[
            pltpu.VMEM((NB, NC, TI, D), bf16),
            pltpu.VMEM((2 * P, D), bf16),
            pltpu.VMEM((D, 2 * P), bf16),
            pltpu.VMEM((NF, D, FP), bf16),
            pltpu.VMEM((NF, D, FP), bf16),
            pltpu.VMEM((NF, FP, D), bf16),
            pltpu.VMEM((NB, MB, D), bf16),
            pltpu.VMEM((NL, MB, 128), f32),
            pltpu.VMEM((NB, MB, 2 * P), f32),
            pltpu.VMEM((2, MB, 2 * P), bf16),
            pltpu.VMEM((NB, NC, TI, D), f32),
            pltpu.VMEM((NB, NC, TI, 128), f32),
            pltpu.VMEM((2, 8, P), f32),
            pltpu.VMEM((2, 8, P), f32),
            pltpu.VMEM((2, D, 128), f32),
            pltpu.VMEM((2, NF, FP, 128), f32),
            pltpu.VMEM((2, 8, D), f32),
            pltpu.SemaphoreType.DMA((NB,)),
            pltpu.SemaphoreType.DMA((4 + 3 * NF,)),
            pltpu.SemaphoreType.DMA((NB + 2,)),
        ],
        compiler_params=pltpu.CompilerParams(vmem_limit_bytes=100 * 1024 * 1024),
    )(A_Lambda_re, A_Lambda_im, A_log_dt, A_Dskip, B_w_r,
      A_x.reshape(NC, LC, D), A_B_re, A_B_im, A_C_re, A_C_im, B_w_gate, B_w_up, B_w_down)
    return out.reshape(1, S, D)
```

```python
import jax
import jax.numpy as jnp
from jax import lax
import jax.experimental.pallas as pl
import jax.experimental.pallas.tpu as pltpu

S, D, P, F = 2048, 1024, 1024, 3584
NC = 8
LC = S // NC
NB = 8
TI = LC // NB
MB = TI * NC
NL = D // 128
NF = 4
FP = F // NF
FT = FP // 128
XB = NL * MB
AO = XB + 2 * D
N1 = N2 = 256
def run(*gens):
    n = gens[0][1]
    done = [0] * len(gens)
    for s in range(1, n + 1):
        for q, (g, m) in enumerate(gens):
            while done[q] < (s * m + n - 1) // n:
                next(g, None); done[q] += 1
    for g, _ in gens:
        for _ in g: pass
f32, bf16, u32 = jnp.float32, jnp.bfloat16, jnp.uint32
NT_DIMS = (((1,), (1,)), ((), ()))


def _rb(v):
    return v.astype(bf16).astype(f32)


def _unpack(w):
    u = pltpu.bitcast(w, u32)
    return pltpu.bitcast(u << 16, f32), pltpu.bitcast(u & jnp.uint32(0xFFFF0000), f32)


def _kernel(lre_ref, lim_ref, ldt_ref, dsk_ref, wr_ref,
            x_hbm, bre_hbm, bim_hbm, cre_hbm, cim_hbm, wg_hbm, wu_hbm, wd_hbm,
            o_hbm,
            x_v, b_v, c_v, c2_v, wg_v, wu_v, wd_v, xp_v, t_v, bu_v, h_v, o_v, r_v, st_v, lam_v,
            acc_v, xs_v, a_v, sem_x, sem_w, sem_o):
    def x_cp(k):
        return pltpu.make_async_copy(x_hbm.at[:, pl.ds(k * TI, TI), :], x_v.at[k], sem_x.at[k])

    def o_cp(k):
        return pltpu.make_async_copy(o_v.at[k], o_hbm.at[:, pl.ds(k * TI, TI), :], sem_o.at[k])

    w_cps = [
        pltpu.make_async_copy(bre_hbm, b_v.at[pl.ds(0, P)], sem_w.at[0]),
        pltpu.make_async_copy(bim_hbm, b_v.at[pl.ds(P, P)], sem_w.at[1]),
        pltpu.make_async_copy(cre_hbm, c_v.at[:, pl.ds(0, P)], sem_w.at[2]),
        pltpu.make_async_copy(cim_hbm, c_v.at[:, pl.ds(P, P)], sem_w.at[3]),
    ]

    def wg_cp(i):
        return pltpu.make_async_copy(wg_hbm.at[:, pl.ds(i * FP, FP)], wg_v.at[i], sem_w.at[4 + i])

    def wu_cp(i):
        return pltpu.make_async_copy(wu_hbm.at[:, pl.ds(i * FP, FP)], wu_v.at[i], sem_w.at[4 + NF + i])

    def wd_cp(i):
        return pltpu.make_async_copy(wd_hbm.at[pl.ds(i * FP, FP)], wd_v.at[i], sem_w.at[4 + 2 * NF + i])

    x_cp(0).start()
    w_cps[0].start()
    w_cps[1].start()
    x_cp(1).start()

    row = lambda ref: ref[...].astype(f32).reshape(1, D)
    lre, lim = row(lre_ref), row(lim_ref)
    dt = _rb(jnp.exp(row(ldt_ref)))
    dsk, wr = row(dsk_ref), row(wr_ref)
    mag = jnp.exp(dt * lre)
    ar, ai = mag * jnp.cos(dt * lim), mag * jnp.sin(dt * lim)
    den = lre * lre + lim * lim
    cr = 2.0 * ((ar - 1.0) * lre + ai * lim) / den
    ci = 2.0 * (ai * lre - (ar - 1.0) * lim) / den
    lam_v[0] = jnp.broadcast_to(ar, (8, P))
    lam_v[1] = jnp.broadcast_to(ai, (8, P))
    st_v[...] = jnp.zeros(st_v.shape, f32)

    def ln(k):
        for c in range(NC):
            x = x_v[k, c].astype(f32)
            m = jnp.mean(x, axis=-1, keepdims=True)
            xc = x - m
            v = _rb(jnp.mean(xc * xc, axis=-1, keepdims=True))
            sd = _rb(jnp.sqrt(_rb(v + 1e-5)))
            xn = _rb(_rb(x - _rb(m)) * (1.0 / sd))
            o_v[k, c] = x + xn + xn * dsk
            r = _rb(jnp.sum(xn * wr, axis=-1, keepdims=True))
            r_v[k, c] = jnp.broadcast_to(r, (TI, 128))
            for g in range(TI // 8):
                for j in range(NL):
                    t_v[pl.ds(j * MB + g * 64 + c * 8, 8), :] = xn[g * 8:(g + 1) * 8, j * 128:(j + 1) * 128]
            yield
        for g in range(TI // 8):
            for s in range(0, 8, 2):
                for j in range(NL):
                    a = t_v[pl.ds(j * MB + g * 64 + s, 8, stride=8), :]
                    b = t_v[pl.ds(j * MB + g * 64 + s + 1, 8, stride=8), :]
                    xp_v[k, pl.ds(g * 64 + s * 8, 16), pl.ds(j * 128, 128)] = (
                        jnp.concatenate([a, b], axis=0).astype(bf16))
            yield

    def mm1(k):
        for n0 in range(0, 2 * P, N1):
            bu_v[k, :, pl.ds(n0, N1)] = lax.dot_general(xp_v[k], b_v[pl.ds(n0, N1), :], NT_DIMS, preferred_element_type=f32)
            yield

    def scan(k, slot=None):
        G = 4
        for j0 in range(0, NL, G):
            js = range(j0, j0 + G)
            lr = [lam_v[0, :, pl.ds(j * 128, 128)] for j in js]
            li = [lam_v[1, :, pl.ds(j * 128, 128)] for j in js]
            hr = [st_v[0, :, pl.ds(j * 128, 128)] for j in js]
            hi = [st_v[1, :, pl.ds(j * 128, 128)] for j in js]
            for i in range(0, TI, 2):
                for n, j in enumerate(js):
                    outr, outi = [], []
                    for ii in (i, i + 1):
                        br = bu_v[k, pl.ds(ii * 8, 8), pl.ds(j * 128, 128)]
                        bi = bu_v[k, pl.ds(ii * 8, 8), pl.ds(P + j * 128, 128)]
                        nr = (lr[n] * hr[n] - li[n] * hi[n]) + br
                        ni = (lr[n] * hi[n] + li[n] * hr[n]) + bi
                        hr[n], hi[n] = nr, ni
                        outr.append(nr)
                        outi.append(ni)
                    if slot is not None:
                        h_v[slot, pl.ds(i * 8, 16), pl.ds(j * 128, 128)] = jnp.concatenate(outr, 0).astype(bf16)
                        h_v[slot, pl.ds(i * 8, 16), pl.ds(P + j * 128, 128)] = jnp.concatenate(outi, 0).astype(bf16)
                if i % 8 == 6: yield
            for n, j in enumerate(js):
                st_v[0, :, pl.ds(j * 128, 128)] = hr[n]
                st_v[1, :, pl.ds(j * 128, 128)] = hi[n]

    def scale_c(k):
        for q in range(0, D // NB, 16):
            rows = pl.ds(pl.multiple_of(k * (D // NB) + q, 16), 16)
            a = c_v[rows, pl.ds(0, P)].astype(f32)
            b = c_v[rows, pl.ds(P, P)].astype(f32)
            c2_v[rows, pl.ds(0, P)] = (a * cr - b * ci).astype(bf16)
            c2_v[rows, pl.ds(P, P)] = (-(a * ci + b * cr)).astype(bf16)
            yield

    def carries():
        pr, pi_ = lam_v[0], lam_v[1]
        n = LC
        while n > 1:
            pr, pi_ = pr * pr - pi_ * pi_, 2.0 * pr * pi_
            n //= 2
        er, ei = st_v[0], st_v[1]
        first = lax.broadcasted_iota(jnp.int32, (8, P), 0) == 0
        sr, si = jnp.zeros_like(er), jnp.zeros_like(ei)
        for _ in range(NC - 1):
            tr = er + (pr * sr - pi_ * si)
            ti = ei + (pr * si + pi_ * sr)
            sr = jnp.where(first, 0.0, pltpu.roll(tr, 1, 0))
            si = jnp.where(first, 0.0, pltpu.roll(ti, 1, 0))
        st_v[0] = sr
        st_v[1] = si

    def mm2(k, slot):
        for n0 in range(0, D, N2):
            y = lax.dot_general(h_v[slot], c2_v[pl.ds(n0, N2), :], NT_DIMS, preferred_element_type=f32)
            for j in range(n0 // 128, (n0 + N2) // 128):
                t_v[pl.ds(j * MB, MB), :] = y[:, j * 128 - n0:(j + 1) * 128 - n0]
                for c in range(NC):
                    for g in range(TI // 8):
                        idx = (k, c, pl.ds(g * 8, 8), pl.ds(j * 128, 128))
                        o_v[idx] = o_v[idx] + t_v[pl.ds(j * MB + g * 64 + c, 8, stride=8), :]
            yield

    def route():
        r = r_v[...].reshape(S, 128)
        q = lax.broadcasted_iota(jnp.int32, (S, 128), 0)
        tok = ((q // TI) % NC) * LC + (q // MB) * TI + q % TI
        m0 = jnp.max(r, axis=0, keepdims=True)
        i0 = jnp.min(jnp.where(r == m0, tok, S), axis=0, keepdims=True)
        r1 = jnp.where(tok == i0, -jnp.inf, r)
        m1 = jnp.max(r1, axis=0, keepdims=True)
        i1 = jnp.min(jnp.where((r1 == m1) & (tok != i0), tok, S), axis=0, keepdims=True)
        toks = [jnp.clip(jnp.max(i), 0, S - 1) for i in (i0, i1)]
        for n, t in enumerate(toks):
            c, s = t // LC, t % LC
            pr = (s % TI) * 8 + c
            base = pl.multiple_of((pr // 16) * 16, 16)
            tile = xp_v[s // TI, pl.ds(base, 16), :].astype(f32)
            sel = lax.broadcasted_iota(jnp.int32, (16, D), 0) == pr % 16
            xs = jnp.sum(jnp.where(sel, tile, 0.0), axis=0, keepdims=True)
            xs_v[pl.ds(8 * n, 8), :] = jnp.broadcast_to(xs, (8, D))
        gates = [_rb(jax.nn.sigmoid(m)) for m in (m0, m1)]
        return toks, gates

    def ffn_up(i):
        xs = xs_v[...].astype(bf16)
        for j in range(FT):
            cols = pl.ds(j * 128, 128)
            g = _rb(jnp.dot(xs, wg_v[i, :, cols], preferred_element_type=f32))
            u = _rb(jnp.dot(xs, wu_v[i, :, cols], preferred_element_type=f32))
            a_v[i, :, cols] = (_rb(g * jax.nn.sigmoid(g)) * u).astype(bf16)
            yield

    def ffn_down(i):
        for j in range(0, D, 256):
            cols = pl.ds(j, 256)
            acc_v[:, cols] += jnp.dot(a_v[i], wd_v[i, :, cols], preferred_element_type=f32)
            yield

    with jax.named_scope("s_w0"):
        x_cp(0).wait()
    with jax.named_scope("s_ln0"):
        run((ln(0), NC + TI // 8))
    with jax.named_scope("s_w1"):
        x_cp(1).wait()
        w_cps[0].wait()
        w_cps[1].wait()
    x_cp(2).start()
    w_cps[2].start()
    w_cps[3].start()
    with jax.named_scope("s_mm0"):
        run((mm1(0), 2 * P // N1), (ln(1), NC + TI // 8))
    with jax.named_scope("s_w2"):
        w_cps[2].wait()
        w_cps[3].wait()
    for k in range(3, NB):
        x_cp(k).start()

    def p1(k, carry):
        x_cp(k + 1).wait()

        @pl.when(k >= 3)
        def _():
            wg_cp(k - 3).start()
            wu_cp(k - 3).start()
            wd_cp(k - 3).start()
        run((mm1(k), 2 * P // N1), (ln(k + 1), NC + TI // 8), (scan(k - 1), TI // 4), (scale_c(k), D // NB // 16))
        return carry
    with jax.named_scope('s_p1'):
        lax.fori_loop(1, NB - 1, p1, 0)
    run((mm1(NB - 1), 2 * P // N1), (scan(NB - 2), TI // 4), (scale_c(0), D // NB // 16), (scale_c(NB - 1), D // NB // 16))
    toks, gates = route()
    acc_v[...] = jnp.zeros(acc_v.shape, f32)
    run((scan(NB - 1), TI // 4))
    carries()
    run((scan(0, 0), TI // 4))

    Z = jnp.clip(jnp.max(st_v[0, :, :128]).astype(jnp.int32), 0, 1) // 2
    def p2a(k, carry):
        wg_cp(k).wait()
        wu_cp(k).wait()
        run((mm2(k, k % 2), D // N2), (scan(k + 1, (k + 1) % 2), TI // 4), (ffn_up(k), 7))
        o_cp(k).start()
        return carry
    with jax.named_scope('s_p2a'):
        lax.fori_loop(0, NF, p2a, 0)

    def p2b(k, carry):
        wd_cp(k - NF).wait()
        run((mm2(k, k % 2), D // N2), (scan(k + 1, (k + 1) % 2), TI // 4), (ffn_down(k - NF), 4))
        o_cp(k).start()
        return carry
    with jax.named_scope('s_p2b'):
        lax.fori_loop(NF, NB - 1, p2b, 0)
    wd_cp(NF - 1).wait()
    run((mm2(NB - 1, Z + 1), D // N2), (ffn_down(NF - 1 + Z), 4))
    for k in range(NB - 1):
        o_cp(k).wait()
    sub = lax.broadcasted_iota(jnp.int32, (8, D), 0)
    fix = []
    for n, t in enumerate(toks):
        c, s = t // LC, t % LC
        y = _rb(_rb(acc_v[pl.ds(8 * n, 8), :]) * gates[n][:, :1])
        r0 = pl.multiple_of(((s % TI) // 8) * 8, 8)
        idx = (s // TI, c, pl.ds(r0, 8), slice(None))
        o_v[idx] = o_v[idx] + jnp.where(sub == s % 8, y, 0.0)
        fix.append((s // TI, pltpu.make_async_copy(
            o_v.at[idx], o_hbm.at[c, pl.ds(pl.multiple_of((s // 8) * 8, 8), 8), :], sem_o.at[NB + n]), t // 8))
    o_cp(NB - 1).start()
    do0 = fix[0][0] != NB - 1
    do1 = (fix[1][0] != NB - 1) & (fix[1][2] != fix[0][2])
    pl.when(do0)(lambda: fix[0][1].start())
    pl.when(do1)(lambda: fix[1][1].start())
    pl.when(do0)(lambda: fix[0][1].wait())
    pl.when(do1)(lambda: fix[1][1].wait())
    o_cp(NB - 1).wait()


@jax.jit
def pallas_parallel_sum__ssm_conv_s5__moe_arch_mod__prompt_kernel(
    A_x, A_Lambda_re, A_Lambda_im, A_B_re, A_B_im, A_C_re, A_C_im, A_log_dt, A_Dskip,
    B_x, B_w_r, B_w_gate, B_w_up, B_w_down,
):
    del B_x
    vm = pl.BlockSpec(memory_space=pltpu.VMEM)
    hb = pl.BlockSpec(memory_space=pl.ANY)
    out = pl.pallas_call(
        _kernel,
        out_shape=jax.ShapeDtypeStruct((NC, LC, D), f32),
        in_specs=[vm] * 5 + [hb] * 8,
        out_specs=hb,
        scratch_shapes=[
            pltpu.VMEM((NB, NC, TI, D), bf16),
            pltpu.VMEM((2 * P, D), bf16),
            pltpu.VMEM((D, 2 * P), bf16),
            pltpu.VMEM((D, 2 * P), bf16),
            pltpu.VMEM((NF, D, FP), bf16),
            pltpu.VMEM((NF, D, FP), bf16),
            pltpu.VMEM((NF, FP, D), bf16),
            pltpu.VMEM((NB, MB, D), bf16),
            pltpu.VMEM((NL * MB, 128), f32),
            pltpu.VMEM((NB, MB, 2 * P), f32),
            pltpu.VMEM((2, MB, 2 * P), bf16),
            pltpu.VMEM((NB, NC, TI, D), f32),
            pltpu.VMEM((NB, NC, TI, 128), f32),
            pltpu.VMEM((2, 8, P), f32),
            pltpu.VMEM((2, 8, P), f32),
            pltpu.VMEM((16, D), f32), pltpu.VMEM((16, D), f32), pltpu.VMEM((NF, 16, FP), bf16),
            pltpu.SemaphoreType.DMA((NB,)),
            pltpu.SemaphoreType.DMA((4 + 3 * NF,)),
            pltpu.SemaphoreType.DMA((NB + 2,)),
        ],
        compiler_params=pltpu.CompilerParams(vmem_limit_bytes=100 * 1024 * 1024, flags={"XLA_TPU_EVENLY_DISTRIBUTE_CRITICAL_NODES": True}),
    )(A_Lambda_re, A_Lambda_im, A_log_dt, A_Dskip, B_w_r,
      A_x.reshape(NC, LC, D), A_B_re, A_B_im, A_C_re, A_C_im, B_w_gate, B_w_up, B_w_down)
    return out.reshape(1, S, D)
```
